```python
import jax
import jax.numpy as jnp

def _softmax(x, axis=-1):
    return jax.nn.softmax(x, axis=axis)
def _gelu(x):
    return jax.nn.gelu(x, approximate=True)
def _silu(x):
    return jax.nn.silu(x)
def _sigmoid(x):
    return jax.nn.sigmoid(x)
def _layernorm(x, axis=-1, eps=1e-5):
    m = jnp.mean(x, axis=axis, keepdims=True)
    v = jnp.var(x, axis=axis, keepdims=True)
    return (x - m) / jnp.sqrt(v + eps)
def _scatter_add(tgt, idx, src, axis=0):
    return tgt.at[idx].add(src)
def _segment_sum(src, seg, n):
    return jax.ops.segment_sum(src, seg, n)
class _Rng:
    def __init__(self, key):
        self._k = key
    def _next(self):
        self._k, sub = jax.random.split(self._k)
        return sub
    def normal(self, shape):
        return jax.random.normal(self._next(), shape, dtype=jnp.bfloat16)
    def randint(self, lo, hi, shape):
        return jax.random.randint(self._next(), shape, lo, hi, dtype=jnp.int32)
    def uniform(self, shape, lo=0.0, hi=1.0):
        return jax.random.uniform(self._next(), shape, jnp.bfloat16, lo, hi)
    def permutation(self, n):
        return jax.random.permutation(self._next(), n)


kernel_name = 'recurrent_scan__sliding_block_cached__moe_arch_mod__prompt'

def setup_inputs():
    _rng = _Rng(jax.random.key(int.from_bytes(__import__("os").urandom(4), "little")))
    _w = (lambda a: (lambda t: t.astype(jnp.bfloat16) if jnp.issubdtype(t.dtype, jnp.floating) else t)(jnp.asarray(a)))
    def _A_setup():
        B, Sq, D = 1, 2048, 640
        Hq, Hkv, Sk, Dh = 32, 32, 2048, 192
        assert Hq % Hkv == 0, (Hq, Hkv)
        return {
            "x": _w((lambda *s: _rng.normal(s) * 0.05)(B, Sq, D)),
            "k_cache": _w((lambda *s: _rng.normal(s) * 0.05)(B, Hkv, Sk, Dh)),
            "v_cache": _w((lambda *s: _rng.normal(s) * 0.05)(B, Hkv, Sk, Dh)),
            "wq": _w((lambda *s: _rng.normal(s) * 0.05)(D, Hq * Dh) * (D ** -0.5)),
            "wo": _w((lambda *s: _rng.normal(s) * 0.05)(Hq * Dh, D) * ((Hq * Dh) ** -0.5)),
        }
    _A_in = _A_setup()

    def _B_setup():
        B, S, D, F, C = 1, 2048, 640, 1536, 2
        return {
            "x": _w((lambda *s: _rng.normal(s) * 0.05)(B, S, D)),
            "w_r": _w((lambda *s: _rng.normal(s) * 0.05)(D)),
            "w_gate": _w((lambda *s: _rng.normal(s) * 0.05)(D, F)),
            "w_up": _w((lambda *s: _rng.normal(s) * 0.05)(D, F)),
            "w_down": _w((lambda *s: _rng.normal(s) * 0.05)(F, D)),
        }
    _B_in = _B_setup()

    return {
        "A_x": _A_in["x"],
        "A_k_cache": _A_in["k_cache"],
        "A_v_cache": _A_in["v_cache"],
        "A_wq": _A_in["wq"],
        "A_wo": _A_in["wo"],
        "B_x": _B_in["x"],
        "B_w_r": _B_in["w_r"],
        "B_w_gate": _B_in["w_gate"],
        "B_w_up": _B_in["w_up"],
        "B_w_down": _B_in["w_down"],
    }

def reference(A_x, A_k_cache, A_v_cache, A_wq, A_wo, B_x, B_w_r, B_w_gate, B_w_up, B_w_down):
    def _A_ref(x, k_cache, v_cache, wq, wo):
        B, Sq, D = x.shape
        Hq, Dh = 32, 192
        Hkv, Sk = k_cache.shape[1], k_cache.shape[2]
        W = min(4096, max(256, Sk // 4))
        rep = Hq // Hkv
        q = (lambda x, *d: x.transpose(*d))((x @ wq).reshape(B, Sq, Hq, Dh), 0, 2, 1, 3)
        k = jnp.repeat(k_cache[:, :, Sk - W:, :], rep, axis=1)
        v = jnp.repeat(v_cache[:, :, Sk - W:, :], rep, axis=1)
        scores = jnp.einsum("bhqd,bhkd->bhqk", q, k) * (Dh ** -0.5)
        p = _softmax(scores, axis=-1)
        o = jnp.einsum("bhqk,bhkd->bhqd", p, v)
        return (lambda x, *d: x.transpose(*d))(o, 0, 2, 1, 3).reshape(B, Sq, Hq * Dh) @ wo

    def _B_ref(x, w_r, w_gate, w_up, w_down):
        B, S, D = x.shape
        C = 2
        r = x @ w_r
        idx = jnp.argsort(-r, axis=-1)[:, :C]
        idx_e = jnp.repeat(idx.reshape(B, C, 1), D, axis=2)
        x_sel = jnp.take_along_axis(x, idx_e, axis=1)
        g = _silu(x_sel @ w_gate)
        u = x_sel @ w_up
        y = (g * u) @ w_down
        r_sel = _sigmoid(jnp.take_along_axis(r, idx, axis=1))
        y = y * r_sel.reshape(B, C, 1)
        b_off = (jnp.arange(B) * S).reshape(B, 1)
        flat_idx = (idx + b_off).reshape(B * C)
        zero = (x * 0.0).reshape(B * S, D)
        upd = _scatter_add(zero, flat_idx, y.reshape(B * C, D), axis=0)
        return x + upd.reshape(B, S, D)

    x = A_x
    xn = _layernorm(x, axis=-1)
    s = _A_ref(xn, A_k_cache, A_v_cache, A_wq, A_wo)
    g = _silu(_B_ref(xn, B_w_r, B_w_gate, B_w_up, B_w_down))
    return x + s * g
```

```python
import functools
import jax
import jax.numpy as jnp
from jax import lax
import numpy as np
import jax.experimental.pallas as pl
import jax.experimental.pallas.tpu as pltpu

S, D, H, DH, W, F = 2048, 640, 32, 192, 512, 1536
SK = 2048
LOG2E = 1.4426950408889634
BF = jnp.bfloat16
F32 = jnp.float32
EPS_BF = float(np.asarray(1e-5, dtype=jnp.bfloat16).astype(np.float32))
SC = DH ** -0.5 * LOG2E


def _rb(x):
    return x.astype(BF).astype(F32)


def _layernorm_T(xT):
    xf = xT.astype(F32)
    mean = jnp.sum(xf, axis=0, keepdims=True) * (1.0 / D)
    c = xf - mean
    var = jnp.sum(c * c, axis=0, keepdims=True) * (1.0 / D)
    den = _rb(jnp.sqrt(_rb(_rb(var) + EPS_BF)))
    return (_rb(xf - _rb(mean)) / den).astype(BF)


def _silu(b):
    h = 0.5 * b
    return h * jnp.tanh(h) + h


def make_kernel(MC=512):
    HP = 2
    NM = S // MC
    NP = H // HP
    R = HP * DH

    def kernel(x_hbm, k_hbm, v_hbm, wq_hbm, wo_hbm, wr_ref, wg_hbm, wu_hbm, wd_hbm, o_hbm,
               x_v, xn_v, xnT_v, acc_v, wq_r, wo_r, k_r, v_r, wqT, woT, kN,
               wg_v, wu_v, wd_v, o_v, r_v, xs_v, rs_v, idx_s, sx, sw, sf, so):

        def x_copy(c):
            return pltpu.make_async_copy(x_hbm.at[pl.ds(pl.multiple_of(c * MC, MC), MC)], x_v.at[pl.ds(pl.multiple_of(c * MC, MC), MC)], sx.at[c])

        def w_copies(p, slot):
            return (
                pltpu.make_async_copy(wq_hbm.at[:, pl.ds(pl.multiple_of(p * R, 128), R)], wq_r.at[slot], sw.at[0, slot]),
                pltpu.make_async_copy(k_hbm.at[pl.ds(p * HP, HP), :, pl.ds(SK - W, W)], k_r.at[slot], sw.at[1, slot]),
                pltpu.make_async_copy(v_hbm.at[pl.ds(p * HP, HP), :, pl.ds(SK - W, W)], v_r.at[slot], sw.at[2, slot]),
                pltpu.make_async_copy(wo_hbm.at[pl.ds(pl.multiple_of(p * R, 128), R), :], wo_r.at[slot], sw.at[3, slot]),
            )

        f_copies = (
            pltpu.make_async_copy(wg_hbm, wg_v, sf.at[0]),
            pltpu.make_async_copy(wu_hbm, wu_v, sf.at[1]),
            pltpu.make_async_copy(wd_hbm, wd_v, sf.at[2]),
        )

        def o_copy(c):
            return pltpu.make_async_copy(o_v.at[pl.ds(pl.multiple_of(c * MC, MC), MC)], o_hbm.at[pl.ds(pl.multiple_of(c * MC, MC), MC)], so.at[c])

        x_copy(0).start()
        w0 = w_copies(0, 0)
        w0[0].start()
        w0[1].start()
        for c in range(1, NM):
            x_copy(c).start()
        w0[2].start()
        w0[3].start()

        def ln_chunk(c, carry):
            x_copy(c).wait()
            rows = pl.ds(pl.multiple_of(c * MC, MC), MC)
            xnT = _layernorm_T(x_v[rows, :].T)
            xnT_v[c] = xnT
            xn_v[rows, :] = xnT.T
            r_v[c] = jnp.dot(wrp, xnT, preferred_element_type=F32)[0:8]
            return carry

        def stQ(c):
            qT = jnp.dot(wqT[...], xnT_v[c], preferred_element_type=F32)
            return (qT * SC).astype(BF)

        def stS(qT, h):
            return jnp.dot(kN[h], qT[h * DH:(h + 1) * DH], preferred_element_type=F32)

        def stP(sT, h, slot):
            m = jnp.max(sT, axis=0, keepdims=True)
            e = jnp.exp2(sT - m)
            l = jnp.sum(e, axis=0, keepdims=True)
            oT = jnp.dot(v_r[slot, h], e.astype(BF), preferred_element_type=F32)
            return (oT * (1.0 / l)).astype(BF)

        def stO(c, outs):
            oT2 = jnp.concatenate(outs, axis=0)
            acc_v[c] += jnp.dot(woT[...], oT2, preferred_element_type=F32)

        def epi_chunk(c, carry):
            rows = pl.ds(pl.multiple_of(c * MC, MC), MC)
            s = acc_v[c].astype(BF).T.astype(F32)
            g = _silu(xn_v[rows, :].astype(F32))
            o_v[rows, :] = (x_v[rows, :].astype(F32) + s * g).astype(BF)
            o_copy(c).start()
            return carry

        def route_a():
            r = _rb(jnp.concatenate([r_v[c, 0:1, :] for c in range(NM)], axis=1))
            pos = lax.broadcasted_iota(jnp.int32, (1, S), 1).astype(F32)
            m0 = jnp.max(r, axis=-1, keepdims=True)
            i0 = jnp.min(jnp.where(r == m0, pos, float(S)), axis=-1, keepdims=True)
            r1 = jnp.where(pos == i0, -jnp.inf, r)
            m1 = jnp.max(r1, axis=-1, keepdims=True)
            i1 = jnp.min(jnp.where(r1 == m1, pos, float(S)), axis=-1, keepdims=True)
            i0 = jnp.clip(i0[0, 0].astype(jnp.int32), 0, S - 1)
            i1 = jnp.clip(i1[0, 0].astype(jnp.int32), 0, S - 1)
            idx_s[0] = i0
            idx_s[1] = i1
            b0 = pl.multiple_of((i0 // 16) * 16, 16)
            b1 = pl.multiple_of((i1 // 16) * 16, 16)
            sub = lax.broadcasted_iota(jnp.int32, (16, D), 0)
            blk0 = xn_v[pl.ds(b0, 16), :].astype(F32)
            blk1 = xn_v[pl.ds(b1, 16), :].astype(F32)
            x0 = jnp.sum(jnp.where(sub == (i0 - b0), blk0, 0.0), axis=0, keepdims=True)
            x1 = jnp.sum(jnp.where(sub == (i1 - b1), blk1, 0.0), axis=0, keepdims=True)
            xs_v[...] = jnp.where(sub == 0, x0, jnp.where(sub == 1, x1, 0.0)).astype(BF)
            sub1 = lax.broadcasted_iota(jnp.int32, (16, 128), 0)
            rs_v[...] = _rb(jax.nn.sigmoid(jnp.where(sub1 == 0, m0, m1)))

        def route_b():
            xs = xs_v[...]
            gg = _rb(jnp.dot(xs, wg_v[...], preferred_element_type=F32))
            uu = _rb(jnp.dot(xs, wu_v[...], preferred_element_type=F32))
            hh = (_rb(gg * _rb(jax.nn.sigmoid(gg))) * uu).astype(BF)
            yy = _rb(jnp.dot(hh, wd_v[...], preferred_element_type=F32))
            yy = _rb(yy * rs_v[:, 0:1])
            i0 = idx_s[0]
            i1 = idx_s[1]
            b0 = pl.multiple_of((i0 // 16) * 16, 16)
            b1 = pl.multiple_of((i1 // 16) * 16, 16)
            sub = lax.broadcasted_iota(jnp.int32, (16, D), 0)
            blk0 = xn_v[pl.ds(b0, 16), :].astype(F32)
            xn_v[pl.ds(b0, 16), :] = jnp.where(sub == (i0 - b0), blk0 + yy[0:1], blk0).astype(BF)
            blk1 = xn_v[pl.ds(b1, 16), :].astype(F32)
            xn_v[pl.ds(b1, 16), :] = jnp.where(sub == (i1 - b1), blk1 + yy[1:2], blk1).astype(BF)

        if True:
            wrp = jnp.where(lax.broadcasted_iota(jnp.int32, (16, D), 0) == 0,
                            wr_ref[...].astype(F32), 0.0).astype(BF)
            acc_v[...] = jnp.zeros_like(acc_v)
            lax.fori_loop(0, NM, ln_chunk, 0)
            for cp in f_copies:
                cp.start()
            route_a()

        def step(p, carry):
            slot = p % 2
            for cp in w_copies(p, slot):
                cp.wait()

            @pl.when(p + 1 < NP)
            def _():
                for cp in w_copies(p + 1, 1 - slot):
                    cp.start()

            wqT[...] = wq_r[slot].T
            for h in range(HP):
                kN[h] = k_r[slot, h].T
            woT[...] = wo_r[slot].T
            qT = stQ(0)
            prev = None
            for c in range(NM):
                ss = [stS(qT, h) for h in range(HP)]
                if c + 1 < NM:
                    qT = stQ(c + 1)
                o0 = stP(ss[0], 0, slot)
                if prev is not None:
                    stO(c - 1, prev)
                o1 = stP(ss[1], 1, slot)
                prev = [o0, o1]
            stO(NM - 1, prev)
            return carry

        if True:
            lax.fori_loop(0, NP, step, 0)
        if True:
            for cp in f_copies:
                cp.wait()
            route_b()
        if True:
            lax.fori_loop(0, NM, epi_chunk, 0)
        if True:
            for c in range(NM):
                o_copy(c).wait()

    def call(x, k, v, wq, wo, wr, wg, wu, wd):
        any_spec = pl.BlockSpec(memory_space=pl.ANY)
        return pl.pallas_call(
            kernel,
            in_specs=[any_spec] * 5 + [pl.BlockSpec(memory_space=pltpu.VMEM)] + [any_spec] * 3,
            out_specs=any_spec,
            out_shape=jax.ShapeDtypeStruct((S, D), BF),
            scratch_shapes=[
                pltpu.VMEM((S, D), BF),
                pltpu.VMEM((S, D), BF),
                pltpu.VMEM((NM, D, MC), BF),
                pltpu.VMEM((NM, D, MC), F32),
                pltpu.VMEM((2, D, R), BF),
                pltpu.VMEM((2, R, D), BF),
                pltpu.VMEM((2, HP, DH, W), BF),
                pltpu.VMEM((2, HP, DH, W), BF),
                pltpu.VMEM((R, D), BF),
                pltpu.VMEM((D, R), BF),
                pltpu.VMEM((HP, W, DH), BF),
                pltpu.VMEM((D, F), BF),
                pltpu.VMEM((D, F), BF),
                pltpu.VMEM((F, D), BF),
                pltpu.VMEM((S, D), BF),
                pltpu.VMEM((NM, 8, MC), F32),
                pltpu.VMEM((16, D), BF),
                pltpu.VMEM((16, 128), F32),
                pltpu.SMEM((2,), jnp.int32),
                pltpu.SemaphoreType.DMA((NM,)),
                pltpu.SemaphoreType.DMA((4, 2)),
                pltpu.SemaphoreType.DMA((3,)),
                pltpu.SemaphoreType.DMA((NM,)),
            ],
            compiler_params=pltpu.CompilerParams(
                vmem_limit_bytes=100 * 1024 * 1024,
            ),
        )(x, k, v, wq, wo, wr, wg, wu, wd)

    def fn(A_x, A_k_cache, A_v_cache, A_wq, A_wo, B_x, B_w_r, B_w_gate, B_w_up, B_w_down):
        out = call(A_x.reshape(S, D), A_k_cache.transpose(0, 1, 3, 2).reshape(H, DH, SK),
                   A_v_cache.transpose(0, 1, 3, 2).reshape(H, DH, SK), A_wq, A_wo, B_w_r.reshape(1, D),
                   B_w_gate, B_w_up, B_w_down)
        return out.reshape(1, S, D)

    return fn


_IMPL = make_kernel()


@jax.jit
def pallas_recurrent_scan__sliding_block_cached__moe_arch_mod__prompt_kernel(
    A_x, A_k_cache, A_v_cache, A_wq, A_wo, B_x, B_w_r, B_w_gate, B_w_up, B_w_down,
):
    return _IMPL(A_x, A_k_cache, A_v_cache, A_wq, A_wo, B_x, B_w_r, B_w_gate, B_w_up, B_w_down)
```

```python
import jax
import jax.numpy as jnp
from jax import lax
import numpy as np
import jax.experimental.pallas as pl
import jax.experimental.pallas.tpu as pltpu

S, D, H, DH, W, F = 2048, 640, 32, 192, 512, 1536
SK = 2048
LOG2E = 1.4426950408889634
BF = jnp.bfloat16
F32 = jnp.float32
EPS_BF = float(np.asarray(1e-5, dtype=jnp.bfloat16).astype(np.float32))
SC = DH ** -0.5 * LOG2E


def _rb(x):
    return x.astype(BF).astype(F32)


def _silu(b):
    h = 0.5 * b
    return h * jnp.tanh(h) + h


def _layernorm_rows(xb):
    xf = xb.astype(F32)
    mean = jnp.sum(xf, axis=-1, keepdims=True) * (1.0 / D)
    c = xf - mean
    var = jnp.sum(c * c, axis=-1, keepdims=True) * (1.0 / D)
    den = _rb(jnp.sqrt(_rb(_rb(var) + EPS_BF)))
    return _rb(_rb(xf - _rb(mean)) / den)


def make_kernel(MC=512, HP=4, EC=256, seq='S0 S1 S2 S3 Q P0 P1 O P2 P3',
                flags={'XLA_TPU_FORCE_LP_LLO_SCHEDULER': True}):
    NM = S // MC
    NP = H // HP
    R = HP * DH
    TPC = MC // 128
    NE = MC // EC

    def kernel(x_hbm, k_hbm, v_hbm, wq_hbm, wo_hbm, wr_ref, wg_hbm, wu_hbm, wd_hbm, o_hbm,
               x_v, xnT_v, acc_v, wq_r, wo_r, k_r, v_r, wqT, woT, kN,
               wg_v, wu_v, wd_v, o_v, r_v, xs_v, rs_v, idx_s, sx, sw, sf, so):

        def x_copy(c):
            return pltpu.make_async_copy(x_hbm.at[pl.ds(pl.multiple_of(c * MC, MC), MC)], x_v.at[pl.ds(pl.multiple_of(c * MC, MC), MC)], sx.at[c])

        def w_copies(p, slot):
            return (
                pltpu.make_async_copy(wq_hbm.at[:, pl.ds(pl.multiple_of(p * R, 128), R)], wq_r.at[slot], sw.at[0, slot]),
                pltpu.make_async_copy(k_hbm.at[pl.ds(p * HP, HP), :, pl.ds(SK - W, W)], k_r.at[slot], sw.at[1, slot]),
                pltpu.make_async_copy(v_hbm.at[pl.ds(p * HP, HP), :, pl.ds(SK - W, W)], v_r.at[slot], sw.at[2, slot]),
                pltpu.make_async_copy(wo_hbm.at[pl.ds(pl.multiple_of(p * R, 128), R), :], wo_r.at[slot], sw.at[3, slot]),
            )

        f_copies = (
            pltpu.make_async_copy(wg_hbm, wg_v, sf.at[0]),
            pltpu.make_async_copy(wu_hbm, wu_v, sf.at[1]),
            pltpu.make_async_copy(wd_hbm, wd_v, sf.at[2]),
        )

        def o_copy(c):
            rows = pl.ds(pl.multiple_of(c * EC, EC), EC)
            return pltpu.make_async_copy(o_v.at[rows], o_hbm.at[rows], so.at[c])

        x_copy(0).start()
        w0 = w_copies(0, 0)
        w0[0].start()
        w0[1].start()
        for c in range(1, NM):
            x_copy(c).start()
        w0[2].start()
        w0[3].start()

        def ln_chunk(c, carry):
            x_copy(c).wait()
            xT = x_v[pl.ds(pl.multiple_of(c * MC, MC), MC), :].T
            ones = jnp.ones((16, D), BF)
            mean = jnp.dot(ones, xT, preferred_element_type=F32)[0:1] * (1.0 / D)
            m = _rb(mean)
            t = xT.astype(F32) - m
            dm = m - mean
            var = jnp.sum(t * t, axis=0, keepdims=True) * (1.0 / D) - dm * dm
            for j in range(TPC):
                xnT_v[c * TPC + j] = t[:, j * 128:(j + 1) * 128].astype(BF)
            den = _rb(jnp.sqrt(_rb(_rb(var) + EPS_BF)))
            inv = 1.0 / den
            for j in range(TPC):
                sl = slice(j * 128, (j + 1) * 128)
                xn = (xnT_v[c * TPC + j].astype(F32) * inv[:, sl]).astype(BF)
                xnT_v[c * TPC + j] = xn
                r_v[c, :, sl] = jnp.dot(wrp, xn, preferred_element_type=F32)[0:8]
            return carry

        def xn_cols(t0, n):
            return jnp.concatenate([xnT_v[t0 + j] for j in range(n)], axis=1)

        def stQ(c):
            qT = jnp.dot(wqT[...], xn_cols(c * TPC, TPC), preferred_element_type=F32)
            return (qT * SC).astype(BF)

        def stS(qT, h):
            return jnp.dot(kN[h], qT[h * DH:(h + 1) * DH], preferred_element_type=F32)

        def stP(sT, h, slot):
            m = jnp.max(sT, axis=0, keepdims=True)
            e = jnp.exp2(sT - m)
            l = jnp.sum(e, axis=0, keepdims=True)
            oT = jnp.dot(v_r[slot, h], e.astype(BF), preferred_element_type=F32)
            return (oT * (1.0 / l)).astype(BF)

        def stO(c, outs):
            oT2 = jnp.concatenate(outs, axis=0)
            res = jnp.dot(woT[...], oT2, preferred_element_type=F32)
            for e in range(NE):
                acc_v[c * NE + e] += res[:, e * EC:(e + 1) * EC]

        def epi_sub(e):
            tpe = EC // 128
            g = _silu(xn_cols(e * tpe, tpe).astype(F32))
            sg = (acc_v[e] * g).astype(BF).T
            rows = pl.ds(pl.multiple_of(e * EC, EC), EC)
            o_v[rows, :] = (x_v[rows, :].astype(F32) + sg.astype(F32)).astype(BF)
            o_copy(e).start()

        def route_a():
            r = _rb(jnp.concatenate([r_v[c, 0:1, :] for c in range(NM)], axis=1))
            pos = lax.broadcasted_iota(jnp.int32, (1, S), 1).astype(F32)
            m0 = jnp.max(r, axis=-1, keepdims=True)
            i0 = jnp.min(jnp.where(r == m0, pos, float(S)), axis=-1, keepdims=True)
            r1 = jnp.where(pos == i0, -jnp.inf, r)
            m1 = jnp.max(r1, axis=-1, keepdims=True)
            i1 = jnp.min(jnp.where(r1 == m1, pos, float(S)), axis=-1, keepdims=True)
            i0 = jnp.clip(i0[0, 0].astype(jnp.int32), 0, S - 1)
            i1 = jnp.clip(i1[0, 0].astype(jnp.int32), 0, S - 1)
            idx_s[0] = i0
            idx_s[1] = i1
            b0 = pl.multiple_of((i0 // 16) * 16, 16)
            b1 = pl.multiple_of((i1 // 16) * 16, 16)
            sub = lax.broadcasted_iota(jnp.int32, (16, D), 0)
            blk0 = _layernorm_rows(x_v[pl.ds(b0, 16), :])
            blk1 = _layernorm_rows(x_v[pl.ds(b1, 16), :])
            x0 = jnp.sum(jnp.where(sub == (i0 - b0), blk0, 0.0), axis=0, keepdims=True)
            x1 = jnp.sum(jnp.where(sub == (i1 - b1), blk1, 0.0), axis=0, keepdims=True)
            xs_v[...] = jnp.where(sub == 0, x0, jnp.where(sub == 1, x1, 0.0)).astype(BF)
            sub1 = lax.broadcasted_iota(jnp.int32, (16, 128), 0)
            rs_v[...] = _rb(jax.nn.sigmoid(jnp.where(sub1 == 0, m0, m1)))

        def route_b():
            xs = xs_v[...]
            gg = _rb(jnp.dot(xs, wg_v[...], preferred_element_type=F32))
            uu = _rb(jnp.dot(xs, wu_v[...], preferred_element_type=F32))
            hh = (_rb(gg * _rb(jax.nn.sigmoid(gg))) * uu).astype(BF)
            yy = _rb(jnp.dot(hh, wd_v[...], preferred_element_type=F32))
            yy = _rb(yy * rs_v[:, 0:1])
            lane = lax.broadcasted_iota(jnp.int32, (D, 128), 1)
            for n in range(2):
                i = idx_s[n]
                t = i // 128
                yT = jnp.broadcast_to(yy[n:n + 1], (128, D)).T
                xt = xnT_v[t].astype(F32)
                xnT_v[t] = jnp.where(lane == i - t * 128, xt + yT, xt).astype(BF)

        wrp = jnp.where(lax.broadcasted_iota(jnp.int32, (16, D), 0) == 0,
                        wr_ref[...].astype(F32)[None, :], 0.0).astype(BF)
        acc_v[...] = jnp.zeros_like(acc_v)
        lax.fori_loop(0, NM, ln_chunk, 0)
        for cp in f_copies:
            cp.start()
        route_a()

        def step(p, carry):
            slot = p % 2
            for cp in w_copies(p, slot):
                cp.wait()

            @pl.when(p + 1 < NP)
            def _():
                for cp in w_copies(p + 1, 1 - slot):
                    cp.start()

            wqT[...] = wq_r[slot].T
            for h in range(HP):
                kN[h] = k_r[slot, h].T
            woT[...] = wo_r[slot].T
            qT = stQ(0)
            prev = None
            for c in range(NM):
                ss = [None] * HP
                outs = [None] * HP
                qn = None
                for tok in seq.split():
                    if tok[0] == 'S':
                        ss[int(tok[1])] = stS(qT, int(tok[1]))
                    elif tok[0] == 'P':
                        outs[int(tok[1])] = stP(ss[int(tok[1])], int(tok[1]), slot)
                    elif tok == 'Q':
                        if c + 1 < NM:
                            qn = stQ(c + 1)
                    elif tok == 'O':
                        if prev is not None:
                            stO(c - 1, prev)
                    elif tok == 'N':
                        stO(c, outs)
                qT = qn
                prev = outs
            if 'N' not in seq:
                stO(NM - 1, prev)
            return carry

        lax.fori_loop(0, NP, step, 0)
        e0 = idx_s[0] // EC
        e1 = idx_s[1] // EC

        def epi_plain(e, carry):
            @pl.when(jnp.logical_and(e != e0, e != e1))
            def _():
                epi_sub(e)
            return carry

        lax.fori_loop(0, NM * NE, epi_plain, 0)
        for cp in f_copies:
            cp.wait()
        route_b()

        def epi_routed(n, carry):
            @pl.when(jnp.logical_or(n == 0, e1 != e0))
            def _():
                epi_sub(jnp.where(n == 0, e0, e1))
            return carry

        lax.fori_loop(0, 2, epi_routed, 0)
        for c in range(NM * NE):
            o_copy(c).wait()

    def call(x, k, v, wq, wo, wr, wg, wu, wd):
        any_spec = pl.BlockSpec(memory_space=pl.ANY)
        return pl.pallas_call(
            kernel,
            in_specs=[any_spec] * 5 + [pl.BlockSpec(memory_space=pltpu.VMEM)] + [any_spec] * 3,
            out_specs=any_spec,
            out_shape=jax.ShapeDtypeStruct((S, D), BF),
            scratch_shapes=[
                pltpu.VMEM((S, D), BF),
                pltpu.VMEM((S // 128, D, 128), BF),
                pltpu.VMEM((NM * NE, D, EC), F32),
                pltpu.VMEM((2, D, R), BF),
                pltpu.VMEM((2, R, D), BF),
                pltpu.VMEM((2, HP, DH, W), BF),
                pltpu.VMEM((2, HP, DH, W), BF),
                pltpu.VMEM((R, D), BF),
                pltpu.VMEM((D, R), BF),
                pltpu.VMEM((HP, W, DH), BF),
                pltpu.VMEM((D, F), BF),
                pltpu.VMEM((D, F), BF),
                pltpu.VMEM((F, D), BF),
                pltpu.VMEM((S, D), BF),
                pltpu.VMEM((NM, 8, MC), F32),
                pltpu.VMEM((16, D), BF),
                pltpu.VMEM((16, 128), F32),
                pltpu.SMEM((2,), jnp.int32),
                pltpu.SemaphoreType.DMA((NM,)),
                pltpu.SemaphoreType.DMA((4, 2)),
                pltpu.SemaphoreType.DMA((3,)),
                pltpu.SemaphoreType.DMA((NM * NE,)),
            ],
            compiler_params=pltpu.CompilerParams(
                vmem_limit_bytes=100 * 1024 * 1024, flags=flags,
            ),
        )(x, k, v, wq, wo, wr, wg, wu, wd)

    def fn(A_x, A_k_cache, A_v_cache, A_wq, A_wo, B_x, B_w_r, B_w_gate, B_w_up, B_w_down):
        out = call(A_x.reshape(S, D), A_k_cache.transpose(0, 1, 3, 2).reshape(H, DH, SK),
                   A_v_cache.transpose(0, 1, 3, 2).reshape(H, DH, SK), A_wq, A_wo, B_w_r,
                   B_w_gate, B_w_up, B_w_down)
        return out.reshape(1, S, D)

    return fn


_IMPL = make_kernel()


@jax.jit
def pallas_recurrent_scan__sliding_block_cached__moe_arch_mod__prompt_kernel(
    A_x, A_k_cache, A_v_cache, A_wq, A_wo, B_x, B_w_r, B_w_gate, B_w_up, B_w_down,
):
    return _IMPL(A_x, A_k_cache, A_v_cache, A_wq, A_wo, B_x, B_w_r, B_w_gate, B_w_up, B_w_down)
```
